```python
import os as _os
_os.environ.setdefault("JAX_PLATFORMS", "cpu")
import jax
import jax.numpy as jnp

def _softmax(x, axis=-1):
    return jax.nn.softmax(x, axis=axis)
def _gelu(x):
    return jax.nn.gelu(x, approximate=True)
def _silu(x):
    return jax.nn.silu(x)
def _sigmoid(x):
    return jax.nn.sigmoid(x)
def _layernorm(x, axis=-1, eps=1e-5):
    m = jnp.mean(x, axis=axis, keepdims=True)
    v = jnp.var(x, axis=axis, keepdims=True)
    return (x - m) / jnp.sqrt(v + eps)
def _scatter_add(tgt, idx, src, axis=0):
    return tgt.at[idx].add(src)
def _segment_sum(src, seg, n):
    return jax.ops.segment_sum(src, seg, n)
class _Rng:
    def __init__(self, key):
        self._k = key
    def _next(self):
        self._k, sub = jax.random.split(self._k)
        return sub
    def normal(self, shape):
        return jax.random.normal(self._next(), shape, dtype=jnp.bfloat16)
    def randint(self, lo, hi, shape):
        return jax.random.randint(self._next(), shape, lo, hi, dtype=jnp.int32)
    def uniform(self, shape, lo=0.0, hi=1.0):
        return jax.random.uniform(self._next(), shape, jnp.bfloat16, lo, hi)
    def permutation(self, n):
        return jax.random.permutation(self._next(), n)


kernel_name = 'sequential_preLN__sliding_local_dilated__dense_activation_relu__prompt'

def setup_inputs():
    _rng = _Rng(jax.random.key(int.from_bytes(__import__("os").urandom(4), "little")))
    _w = (lambda a: (lambda t: t.astype(jnp.bfloat16) if jnp.issubdtype(t.dtype, jnp.floating) else t)(jnp.asarray(a)))
    def _A_setup():
        B, S, D = 1, 2048, 1024
        return {
            "x": _w((lambda *s: _rng.normal(s) * 0.05)(B, S, D)),
            "wqkv": _w((lambda *s: _rng.normal(s) * 0.05)(D, 3 * D)),
            "wo": _w((lambda *s: _rng.normal(s) * 0.05)(D, D)),
        }
    _A_in = _A_setup()

    def _B_setup():
        B, S, D, Dff = 1, 2048, 1024, 3584
        return {
            "x": _w((lambda *s: _rng.normal(s) * 0.05)(B, S, D)),
            "w1": _w((lambda *s: _rng.normal(s) * 0.05)(D, Dff)),
            "w2": _w((lambda *s: _rng.normal(s) * 0.05)(Dff, D)),
        }
    _B_in = _B_setup()

    return {
        "A_x": _A_in["x"],
        "A_wqkv": _A_in["wqkv"],
        "A_wo": _A_in["wo"],
        "B_x": _B_in["x"],
        "B_w1": _B_in["w1"],
        "B_w2": _B_in["w2"],
    }

def reference(A_x, A_wqkv, A_wo, B_x, B_w1, B_w2):
    def _A_ref(x, wqkv, wo):
        B, S, D = x.shape
        H = 32; Dh = D // H
        W, dil = 8, 2
        qkv = (lambda x, *d: x.transpose(*d))((x @ wqkv).reshape(B, S, 3, H, Dh), 2, 0, 3, 1, 4)
        q, k, v = qkv[0], qkv[1], qkv[2]
        scale = Dh ** -0.5
        pos = jnp.arange(S)
        off = jnp.arange(W) * dil
        idx = pos[:, None] - off[None, :]
        mask = idx >= 0
        idx_c = jnp.where(mask, idx, 0).reshape(-1)
        kg = k[:, :, idx_c, :].reshape(B, H, S, W, Dh)
        vg = v[:, :, idx_c, :].reshape(B, H, S, W, Dh)
        logits = jnp.einsum("bhsd,bhswd->bhsw", q, kg) * scale
        logits = jnp.where(mask[None, None, :, :], logits, -1e9)
        attn = _softmax(logits, axis=-1)
        o = jnp.einsum("bhsw,bhswd->bhsd", attn, vg)
        return (lambda x, *d: x.transpose(*d))(o, 0, 2, 1, 3).reshape(B, S, D) @ wo

    def _B_ref(x, w1, w2):
        h = jnp.einsum("bsd,df->bsf", x, w1)
        zero = jnp.zeros_like(h)
        h = jnp.maximum(h, zero)
        return jnp.einsum("bsf,fd->bsd", h, w2)

    x = A_x
    h = x + _A_ref(_layernorm(x, axis=-1), A_wqkv, A_wo)
    h2 = h + _B_ref(_layernorm(h, axis=-1), B_w1, B_w2)
    return h2
```

```python
import functools

import jax
import jax.numpy as jnp
import numpy as np
from jax import lax
from jax.experimental import pallas as pl
from jax.experimental.pallas import tpu as pltpu

S, D, F = 2048, 1024, 3584
H, DH = 32, 32
NW, DIL = 8, 2
HALO = 16
EPS = 1e-5
NEG = -1e9
SCALE = DH ** -0.5
LANES = 128
NT = D // LANES
PITCH = DH + 1

T = 256
R = 8
RP = 16
LNR = 8
FC = 512
MR = 128
KK = 512
NTILES = S // T


def _layernorm(x):
    m = jnp.mean(x, axis=-1, keepdims=True)
    xc = x - m
    v = jnp.mean(xc * xc, axis=-1, keepdims=True)
    return xc * lax.rsqrt(v + EPS)


def _kernel(zero_ref, x_hbm, wqkv_hbm, wo_hbm, w1_hbm, w2_hbm, out_hbm,
            x_all, wraw, wo_raw, s1, wq, wk, wv, wo, w1, w2,
            xn0, xn1, qb, kb, q0b, k0b, vb, pb, o_all, hn, hc, hln, h1, out_all,
            sem_x, sem_w, sem_out):
    f32 = jnp.float32
    bf16 = jnp.bfloat16
    P = functools.partial
    xn = (xn0, xn1)
    nblk = [0]

    def region(fn):
        nblk[0] += 1
        pl.when(zero_ref[0] < nblk[0])(fn)

    def x_copy(i):
        return pltpu.make_async_copy(x_hbm.at[pl.ds(i * T, T)], x_all.at[pl.ds(i * T, T)], sem_x.at[i])

    def wqkv_copy(g, rb):
        return pltpu.make_async_copy(
            wqkv_hbm.at[pl.ds(rb * 256, 256), pl.ds(g * D, D)],
            wraw.at[g, pl.ds(rb * 256, 256)], sem_w.at[g * 4 + rb])

    FS = F // (NTILES - 1)

    def bulk_copies(i):
        sl = pl.ds(i * FS, FS)
        return [pltpu.make_async_copy(w1_hbm.at[:, sl], w1.at[:, sl], sem_w.at[12]),
                pltpu.make_async_copy(w2_hbm.at[sl], w2.at[sl], sem_w.at[13])]

    def wo_copy(t):
        return pltpu.make_async_copy(wo_hbm.at[:, pl.ds(t * LANES, LANES)], wo_raw.at[t], sem_w.at[14 + t])

    chain = [x_copy(0)] + [wqkv_copy(g, rb) for g in range(2) for rb in range(4)] + [x_copy(1)] + [wqkv_copy(2, rb) for rb in range(4)] + [x_copy(2)]
    WIN = 3
    state = {"started": 0}

    def start_next(n=1):
        for _ in range(n):
            if state["started"] < len(chain):
                chain[state["started"]].start()
                state["started"] += 1

    def wait_chain(j):
        chain[j].wait()
        start_next()

    start_next(WIN)

    def rows(i):
        if isinstance(i, int):
            return pl.ds(i * T, T)
        return pl.ds(pl.multiple_of(i * T, T), T)

    def permute_cols(g, rb, dst):
        for t in range(NT):
            a = pltpu.bitcast(wraw[g, rb * 256:(rb + 1) * 256, t * LANES:(t + 1) * LANES], jnp.int32)
            at = a.T
            for hl in range(4):
                h = 4 * t + hl
                s1[rb, h * PITCH:h * PITCH + DH, :] = at[hl * DH:(hl + 1) * DH]
        for c in range(NT):
            parts = [s1[rb, pl.ds(4 * c + dl, H, stride=PITCH), :] for dl in range(4)]
            b = jnp.concatenate(parts, axis=0)
            dst.at[c].bitcast(jnp.int32)[rb * 128:(rb + 1) * 128, :] = b.T

    def permute_wo(t):
        raw32 = wo_raw.at[t].bitcast(jnp.int32)
        wo32 = wo.at[t].bitcast(jnp.int32)
        p = t % 4
        for h in range(H):
            base = (h % 2) * 16 * 17 + (h // 2) * 17
            s1[p, base:base + 16, :] = raw32[16 * h:16 * h + 16, :]
        for c in range(NT):
            for j in range(2):
                ev = s1[p, pl.ds(2 * c + j, 16, stride=17), :]
                od = s1[p, pl.ds(16 * 17 + 2 * c + j, 16, stride=17), :]
                lo = (ev & 0xFFFF) | (od << 16)
                hi = lax.shift_right_logical(ev, 16) | (od & jnp.int32(-65536))
                r0 = (c * LANES + (2 * j) * DH) // 2
                wo32[r0:r0 + 16, :] = lo
                wo32[r0 + 16:r0 + 32, :] = hi

    prev = [None]

    def tie(x, dep):
        zero = lax.shift_right_logical(lax.shift_right_logical(pltpu.bitcast(dep, jnp.int32), 31), 1)
        return pltpu.bitcast(pltpu.bitcast(x, jnp.int32) | zero, f32)

    def ln1_piece(i, r0, n, tied):
        r = slice(i * T + r0, i * T + r0 + n)
        parts = [x_all[r, c * LANES:(c + 1) * LANES].astype(f32) for c in range(NT)]
        s1_ = functools.reduce(lambda a, b: a + b, parts)
        if tied and prev[0] is not None:
            s1_ = tie(s1_, prev[0])
        m = jnp.sum(s1_, axis=-1, keepdims=True) * (1.0 / D)
        ds = [p - m for p in parts]
        s2_ = functools.reduce(lambda a, b: a + b, [d * d for d in ds])
        v = jnp.sum(s2_, axis=-1, keepdims=True) * (1.0 / D)
        rs = lax.rsqrt(v + EPS)
        for c in range(NT):
            xn[i % 2][r0:r0 + n, c * LANES:(c + 1) * LANES] = ds[c] * rs
        prev[0] = jnp.broadcast_to(m, (n, LANES))

    def proj_piece(xr, w, dst, off, c, mi, ki):
        lhs = xr[mi * MR:(mi + 1) * MR, ki * KK:(ki + 1) * KK].astype(bf16)
        r = jnp.dot(lhs, w[c, ki * KK:(ki + 1) * KK, :], preferred_element_type=f32)
        rs = slice(off + mi * MR, off + (mi + 1) * MR)
        if ki == 0:
            dst[c, rs, :] = r
        else:
            dst[c, rs, :] += r

    def proj_pieces(xr, w, dst, off):
        return [P(proj_piece, xr, w, dst, off, c, mi, ki)
                for mi in range(T // MR) for c in range(NT) for ki in range(D // KK)]

    lprev = [None]

    def logits_gen(r0, i, tied=0):
        qr, kr = (q0b, k0b) if i == 0 else (qb, kb)
        qs = [qr[c, r0:r0 + R, :] for c in range(NT)]
        if tied and lprev[0] is not None:
            qs[0] = tie(qs[0], lprev[0])
        accs = []
        for w in range(NW):
            lo = HALO + r0 - DIL * w
            acc = None
            for c in range(NT):
                t = qs[c] * kr[c, lo:lo + R, :]
                acc = t if acc is None else acc + t
            accs.append(acc)
            yield
        accs = [a + pltpu.roll(a, 64, 1) for a in accs]
        if tied == 1:
            lprev[0] = accs[0]
        yield
        accs = [a + pltpu.roll(a, 32, 1) for a in accs]
        yield
        for w in range(NW):
            l = accs[w] * SCALE
            if i * T + r0 - DIL * w < 0:
                pos = r0 + lax.broadcasted_iota(jnp.int32, (R, LANES), 0)
                l = jnp.where(pos >= DIL * w, l, NEG)
            pb[w, r0:r0 + R, :] = l
        if tied == 2:
            lprev[0] = l
        yield
    LOGITS_STEPS = NW + 3

    def pv_gen(r0, i):
        ls = [pb[w, r0:r0 + RP, :] for w in range(NW)]
        m = functools.reduce(jnp.maximum, ls)
        es = [jnp.exp(l - m) for l in ls]
        yield
        s = functools.reduce(lambda a, b: a + b, es)
        inv = 1.0 / s
        ps = [e * inv for e in es]
        yield
        for c in range(NT):
            acc = None
            for w in range(NW):
                lo = HALO + r0 - DIL * w
                t = ps[w] * vb[c, lo:lo + RP, :]
                acc = t if acc is None else acc + t
            o_all[i * T + r0:i * T + r0 + RP, c * LANES:(c + 1) * LANES] = acc
            yield
    PV_STEPS = NT + 2

    def chain_gens(fns):
        for f in fns:
            yield from f()

    def once(f):
        def g():
            f()
            yield
        return g

    def stream(fns, a=0.0, b=1.0):
        return (chain_gens([once(f) for f in fns]), len(fns), a, b)

    def run_interleaved(mm, streams):
        n = len(mm)
        done = [0] * len(streams)
        for j, fn in enumerate(mm):
            fn()
            for si, (g, steps, a, b) in enumerate(streams):
                frac = min(max(((j + 1) / n - a) / (b - a), 0.0), 1.0)
                target = int(round(frac * steps))
                while done[si] < target:
                    next(g)
                    done[si] += 1
        for g, steps, a, b in streams:
            for _ in g:
                raise AssertionError("stream longer than declared")

    def logits_stream(i, a, b):
        n = T // R
        return (chain_gens([P(logits_gen, j * R, i) for j in range(n)]), n * LOGITS_STEPS, a, b)

    def pv_stream(i, a, b):
        n = T // RP
        return (chain_gens([P(pv_gen, j * RP, i) for j in range(n)]), n * PV_STEPS, a, b)

    def ln1_stream(i, a, b):
        prev[0] = None
        return stream([P(ln1_piece, i, r0, LNR, True) for r0 in range(0, T, LNR)], a, b)

    def wo_piece(c, mi, ki, i):
        cols = slice(c * LANES, (c + 1) * LANES)
        if isinstance(i, int):
            src = pl.ds(i * T + mi * MR, MR)
        else:
            src = pl.ds(pl.multiple_of(i * T + mi * MR, MR), MR)
        lhs = o_all[src, ki * KK:(ki + 1) * KK].astype(bf16)
        r = jnp.dot(lhs, wo[c, ki * KK:(ki + 1) * KK, :], preferred_element_type=f32)
        rs = slice(mi * MR, (mi + 1) * MR)
        if ki == 0:
            hn[rs, cols] = x_all[src, cols].astype(f32) + r
        else:
            hn[rs, cols] += r

    def wo_pieces(i):
        return [P(wo_piece, c, mi, ki, i) for mi in range(T // MR) for c in range(NT) for ki in range(D // KK)]

    def ln2_piece(r0):
        hln[r0:r0 + 32, :] = _layernorm(hn[r0:r0 + 32, :])

    def ffn1_chunk(c):
        cols = slice(c * FC, (c + 1) * FC)
        t = jnp.dot(hln[...].astype(bf16), w1[:, cols], preferred_element_type=f32)
        h1[:, cols] = jnp.maximum(t, 0.0).astype(h1.dtype)

    def ffn2_tile(c, i):
        cols = slice(c * LANES, (c + 1) * LANES)
        t = jnp.dot(h1[...].astype(bf16), w2[:, cols], preferred_element_type=f32)
        out_all[rows(i), cols] = (hc[:, cols] + t).astype(bf16)

    def out_copy(i):
        return pltpu.make_async_copy(out_all.at[rows(i)], out_hbm.at[rows(i)], sem_out)

    def k_halo(src):
        for c in range(NT):
            kb[c, :HALO, :] = src[c, T:, :]

    def v_halo():
        for c in range(NT):
            vb[c, :HALO, :] = vb[c, T:, :]

    LSP = [int(v) for v in "0,0,0,0,4".split(",")]

    def part_logits(lo, hi, a=0.0, b=1.0, tied=0):
        lprev[0] = None
        return (chain_gens([P(logits_gen, j * R, 0, tied) for j in range(lo, hi)]), (hi - lo) * LOGITS_STEPS, a, b)

    def v_first():
        for c in range(NT):
            vb[c, :HALO, :] = jnp.broadcast_to(vb[c, HALO:HALO + 1, :], (HALO, LANES))

    def wo_ts(i):
        return [t for t in range(NT) if 1 + t * (NTILES - 2) // NT == i]

    def step_a(i):
        v_halo()
        streams = [logits_stream(i, 0.0, 1.0)]
        if 1 and wo_ts(i):
            streams.append(stream([P(permute_wo, t) for t in wo_ts(i)]))
        run_interleaved(proj_pieces(xn[i % 2], wv, vb, HALO), streams)

    def step_b(i):
        k_halo(k0b if i == 0 else kb)
        x = xn[(i + 1) % 2]
        streams = [pv_stream(i, 0.0, 1.0)]
        if i == 0 and LSP[-1] < T // R:
            streams = [part_logits(LSP[-1], T // R, 0.0, 0.2, 0), pv_stream(i, 0.2, 1.0)]
        if i + 2 < NTILES:
            streams.append(ln1_stream(i + 2, 0.0, 1.0))
        if not 1 and wo_ts(i):
            streams.append(stream([P(permute_wo, t) for t in wo_ts(i)]))
        run_interleaved(proj_pieces(x, wq, qb, 0) + proj_pieces(x, wk, kb, HALO), streams)

    def kpart(xr, w, dst, off, ki):
        return [P(proj_piece, xr, w, dst, off, c, mi, ki) for mi in range(T // MR) for c in range(NT)]

    def block(name, waits, mm, vec):
        for j in waits:
            wait_chain(j)
        if mm:
            region(lambda: run_interleaved(mm, [stream(v) for v in vec]))
        else:
            def plain():
                for v in vec:
                    for f in v:
                        f()
            region(plain)

    pc = lambda g, rb: P(permute_cols, g, rb, (wq, wk, wv)[g])
    assert KK == 512
    for c in range(NT):
        k0b[c, :HALO, :] = jnp.zeros((HALO, LANES), f32)
    x0 = xn[0]
    def chunk_piece(w, dst, off, rb, c2, mi):
        k0 = rb * 256
        lhs = x0[mi * MR:(mi + 1) * MR, k0:k0 + 256].astype(bf16)
        rhs = jnp.concatenate([w[c2, k0:k0 + 256, :], w[c2 + 1, k0:k0 + 256, :]], axis=1)
        r = jnp.dot(lhs, rhs, preferred_element_type=f32)
        rs = slice(off + mi * MR, off + (mi + 1) * MR)
        for j in range(2):
            part = r[:, j * LANES:(j + 1) * LANES]
            if rb == 0:
                dst[c2 + j, rs, :] = part
            else:
                dst[c2 + j, rs, :] += part

    def chunk_mm(n):
        g, rb = divmod(n, 4)
        w, dst, off = ((wq, q0b, 0), (wk, k0b, HALO), (wv, vb, HALO))[g]
        return [P(chunk_piece, w, dst, off, rb, c2, mi) for mi in range(T // MR) for c2 in range(0, NT, 2)]


    block('P0', [0], [], [[P(ln1_piece, 0, r0, 32, False) for r0 in range(0, T, 32)]])
    block('P1', [1], [], [[pc(0, 0)]])
    for n in range(12):
        if n < 7:
            wait_chain(2 + n)
        elif n == 7:
            wait_chain(9)
            wait_chain(10)
        elif n < 11:
            wait_chain(3 + n)
        def blk(n=n):
            st = []
            if n < 11:
                st.append(stream([pc((n + 1) // 4, (n + 1) % 4)]))
            if n >= 8:
                st.append(part_logits(LSP[n - 8], LSP[n - 7]))
            if n == 11:
                st.append(stream([P(ln1_piece, 1, r0, 32, False) for r0 in range(0, T, 32)]))
            run_interleaved(chunk_mm(n) + ([v_first] if n == 11 else []), st)
        region(blk)
    wait_chain(14)
    assert state["started"] == len(chain)

    for i in range(NTILES):
        cps = []
        if i < NTILES - 1:
            cps = bulk_copies(i) + ([x_copy(i + 3)] if i + 3 < NTILES else [])
            cps += [wo_copy(t) for t in range(NT) if (t * (NTILES - 2) // NT) == i]
        for cp in cps:
            cp.start()
        if i > 0:
            region(P(step_a, i))
        if i < NTILES - 1:
            region(P(step_b, i))
        if i + 3 < NTILES:
            x_copy(i + 3).wait()
        for t in range(NT):
            if i < NTILES - 1 and (t * (NTILES - 2) // NT) == i:
                wo_copy(t).wait()

    last = NTILES - 1

    def last_block():
        wp = wo_pieces(0)
        half = len(wp) // 2
        mm = wp[:half + 2] + [P(ln2_piece, r0) for r0 in range(0, T // 2, 32)] + wp[half + 2:] + [P(ln2_piece, r0) for r0 in range(T // 2, T, 32)]
        run_interleaved(mm, [pv_stream(last, 0.0, 0.75)])
    region(last_block)

    pltpu.make_async_copy(w1_hbm, w1, sem_w.at[12]).wait()
    pltpu.make_async_copy(w2_hbm, w2, sem_w.at[13]).wait()

    def body2(i, carry):
        hc[...] = hn[...]
        for c in range(F // FC):
            ffn1_chunk(c)
        for f in wo_pieces(i + 1):
            f()
        for r0 in range(0, T, 32):
            ln2_piece(r0)
        for c in range(NT):
            ffn2_tile(c, i)
        out_copy(i).start()
        return carry

    if 0:
        for j in range(NTILES - 1):
            if 0 == 1:
                region(P(body2, j, None))
            else:
                body2(j, None)
    else:
        lax.fori_loop(0, NTILES - 1, body2, None)
    hc[...] = hn[...]
    for c in range(F // FC):
        ffn1_chunk(c)
    for c in range(NT):
        ffn2_tile(c, last)
    out_copy(last).start()
    pltpu.make_async_copy(out_all, out_hbm, sem_out).wait()


def fused(x, wqkv, wo, w1, w2):
    f32 = jnp.float32
    bf16 = jnp.bfloat16
    any_spec = pl.BlockSpec(memory_space=pl.ANY)
    scratch = [
        pltpu.VMEM((S, D), bf16),
        pltpu.VMEM((3, D, D), bf16),
        pltpu.VMEM((NT, D, LANES), bf16),
        pltpu.VMEM((4, H * PITCH, LANES), jnp.int32),
        pltpu.VMEM((NT, D, LANES), bf16),
        pltpu.VMEM((NT, D, LANES), bf16),
        pltpu.VMEM((NT, D, LANES), bf16),
        pltpu.VMEM((NT, D, LANES), bf16),
        pltpu.VMEM((D, F), bf16),
        pltpu.VMEM((F, D), bf16),
        pltpu.VMEM((T, D), f32),
        pltpu.VMEM((T, D), f32),
        pltpu.VMEM((NT, T, LANES), f32),
        pltpu.VMEM((NT, HALO + T, LANES), f32),
        pltpu.VMEM((NT, T, LANES), f32),
        pltpu.VMEM((NT, HALO + T, LANES), f32),
        pltpu.VMEM((NT, HALO + T, LANES), f32),
        pltpu.VMEM((NW, T, LANES), f32),
        pltpu.VMEM((S, D), f32),
        pltpu.VMEM((T, D), f32),
        pltpu.VMEM((T, D), f32),
        pltpu.VMEM((T, D), f32),
        pltpu.VMEM((T, F), f32 if 1 else bf16),
        pltpu.VMEM((S, D), bf16),
        pltpu.SemaphoreType.DMA((NTILES,)),
        pltpu.SemaphoreType.DMA((22,)),
        pltpu.SemaphoreType.DMA(()),
    ]
    return pl.pallas_call(
        _kernel,
        out_shape=jax.ShapeDtypeStruct((S, D), bf16),
        in_specs=[pl.BlockSpec(memory_space=pltpu.SMEM)] + [any_spec] * 5,
        out_specs=any_spec,
        scratch_shapes=scratch,
        compiler_params=pltpu.CompilerParams(vmem_limit_bytes=110 * 2 ** 20),
        name="fused_block",
    )(np.zeros((1,), np.int32), x, wqkv, wo, w1, w2)


@jax.jit
def pallas_sequential_preLN__sliding_local_dilated__dense_activation_relu__prompt_kernel(
        A_x, A_wqkv, A_wo, B_x, B_w1, B_w2):
    del B_x
    out = fused(A_x.reshape(S, D), A_wqkv, A_wo, B_w1, B_w2)
    return out.reshape(A_x.shape)
```

```python
import functools

import jax
import jax.numpy as jnp
import numpy as np
from jax import lax
from jax.experimental import pallas as pl
from jax.experimental.pallas import tpu as pltpu

S, D, F = 2048, 1024, 3584
H, DH = 32, 32
NW, DIL = 8, 2
HALO = 16
EPS = 1e-5
NEG = -1e9
SCALE = DH ** -0.5
LANES = 128
NT = D // LANES
PITCH = DH + 1

T = 256
R = 8
RP = 16
LNR = 8
FC = 512
MR = 128
KK = 512
NTILES = S // T


def _layernorm(x):
    m = jnp.mean(x, axis=-1, keepdims=True)
    xc = x - m
    v = jnp.mean(xc * xc, axis=-1, keepdims=True)
    return xc * lax.rsqrt(v + EPS)


def _kernel(zero_ref, x_hbm, wqkv_hbm, wo_hbm, w1_hbm, w2_hbm, out_hbm,
            x_all, wraw, wo_raw, s1, wq, wk, wv, wo, w1, w2,
            xn0, xn1, qb, kb, q0b, k0b, vb, pb, o_all, hn, hc, hln, h1, out_all,
            sem_x, sem_w, sem_out):
    f32 = jnp.float32
    bf16 = jnp.bfloat16
    P = functools.partial
    xn = (xn0, xn1)
    nblk = [0]

    def region(fn):
        nblk[0] += 1
        pl.when(zero_ref[0] < nblk[0])(fn)

    def x_copy(i):
        return pltpu.make_async_copy(x_hbm.at[pl.ds(i * T, T)], x_all.at[pl.ds(i * T, T)], sem_x.at[i])

    def wqkv_copy(g, rb):
        return pltpu.make_async_copy(
            wqkv_hbm.at[pl.ds(rb * 256, 256), pl.ds(g * D, D)],
            wraw.at[g, pl.ds(rb * 256, 256)], sem_w.at[g * 4 + rb])

    FS = F // (NTILES - 1)

    def bulk_copies(i):
        sl = pl.ds(i * FS, FS)
        return [pltpu.make_async_copy(w1_hbm.at[:, sl], w1.at[:, sl], sem_w.at[12]),
                pltpu.make_async_copy(w2_hbm.at[sl], w2.at[sl], sem_w.at[13])]

    def wo_copy(t):
        return pltpu.make_async_copy(wo_hbm.at[:, pl.ds(t * LANES, LANES)], wo_raw.at[t], sem_w.at[14 + t])

    chain = [x_copy(0)] + [wqkv_copy(g, rb) for g in range(2) for rb in range(4)] + [x_copy(1)] + [wqkv_copy(2, rb) for rb in range(4)] + [x_copy(2)]
    WIN = 3
    state = {"started": 0}

    def start_next(n=1):
        for _ in range(n):
            if state["started"] < len(chain):
                chain[state["started"]].start()
                state["started"] += 1

    def wait_chain(j):
        chain[j].wait()
        start_next(1 + (WIN - 3 if j == 0 else 0))

    start_next(3)

    def rows(i):
        if isinstance(i, int):
            return pl.ds(i * T, T)
        return pl.ds(pl.multiple_of(i * T, T), T)

    def permute_cols(g, rb, dst):
        for t in range(NT):
            a = pltpu.bitcast(wraw[g, rb * 256:(rb + 1) * 256, t * LANES:(t + 1) * LANES], jnp.int32)
            at = a.T
            for hl in range(4):
                h = 4 * t + hl
                s1[rb, h * PITCH:h * PITCH + DH, :] = at[hl * DH:(hl + 1) * DH]
        for c in range(NT):
            parts = [s1[rb, pl.ds(4 * c + dl, H, stride=PITCH), :] for dl in range(4)]
            b = jnp.concatenate(parts, axis=0)
            dst.at[c].bitcast(jnp.int32)[rb * 128:(rb + 1) * 128, :] = b.T

    def permute_wo(t):
        raw32 = wo_raw.at[t].bitcast(jnp.int32)
        wo32 = wo.at[t].bitcast(jnp.int32)
        p = t % 4
        for h in range(H):
            base = (h % 2) * 16 * 17 + (h // 2) * 17
            s1[p, base:base + 16, :] = raw32[16 * h:16 * h + 16, :]
        for c in range(NT):
            for j in range(2):
                ev = s1[p, pl.ds(2 * c + j, 16, stride=17), :]
                od = s1[p, pl.ds(16 * 17 + 2 * c + j, 16, stride=17), :]
                lo = (ev & 0xFFFF) | (od << 16)
                hi = lax.shift_right_logical(ev, 16) | (od & jnp.int32(-65536))
                r0 = (c * LANES + (2 * j) * DH) // 2
                wo32[r0:r0 + 16, :] = lo
                wo32[r0 + 16:r0 + 32, :] = hi

    prev = [None]

    def tie(x, dep):
        zero = lax.shift_right_logical(lax.shift_right_logical(pltpu.bitcast(dep, jnp.int32), 31), 1)
        return pltpu.bitcast(pltpu.bitcast(x, jnp.int32) | zero, f32)

    def ln1_piece(i, r0, n, tied):
        r = slice(i * T + r0, i * T + r0 + n)
        parts = [x_all[r, c * LANES:(c + 1) * LANES].astype(f32) for c in range(NT)]
        s1_ = functools.reduce(lambda a, b: a + b, parts)
        if tied and prev[0] is not None:
            s1_ = tie(s1_, prev[0])
        m = jnp.sum(s1_, axis=-1, keepdims=True) * (1.0 / D)
        ds = [p - m for p in parts]
        s2_ = functools.reduce(lambda a, b: a + b, [d * d for d in ds])
        v = jnp.sum(s2_, axis=-1, keepdims=True) * (1.0 / D)
        rs = lax.rsqrt(v + EPS)
        for c in range(NT):
            xn[i % 2][r0:r0 + n, c * LANES:(c + 1) * LANES] = ds[c] * rs
        prev[0] = jnp.broadcast_to(m, (n, LANES))

    def proj_piece(xr, w, dst, off, c, mi, ki):
        lhs = xr[mi * MR:(mi + 1) * MR, ki * KK:(ki + 1) * KK].astype(bf16)
        r = jnp.dot(lhs, w[c, ki * KK:(ki + 1) * KK, :], preferred_element_type=f32)
        rs = slice(off + mi * MR, off + (mi + 1) * MR)
        if ki == 0:
            dst[c, rs, :] = r
        else:
            dst[c, rs, :] += r

    def proj_pieces(xr, w, dst, off):
        return [P(proj_piece, xr, w, dst, off, c, mi, ki)
                for mi in range(T // MR) for c in range(NT) for ki in range(D // KK)]

    lprev = [None]

    def logits_gen(r0, i, tied=0):
        qr, kr = (q0b, k0b) if i == 0 else (qb, kb)
        qs = [qr[c, r0:r0 + R, :] for c in range(NT)]
        if tied and lprev[0] is not None:
            qs[0] = tie(qs[0], lprev[0])
        accs = []
        for w in range(NW):
            lo = HALO + r0 - DIL * w
            acc = None
            for c in range(NT):
                t = qs[c] * kr[c, lo:lo + R, :]
                acc = t if acc is None else acc + t
            accs.append(acc)
            yield
        accs = [a + pltpu.roll(a, 64, 1) for a in accs]
        if tied == 1:
            lprev[0] = accs[0]
        yield
        accs = [a + pltpu.roll(a, 32, 1) for a in accs]
        yield
        for w in range(NW):
            l = accs[w] * SCALE
            if i * T + r0 - DIL * w < 0:
                pos = r0 + lax.broadcasted_iota(jnp.int32, (R, LANES), 0)
                l = jnp.where(pos >= DIL * w, l, NEG)
            pb[w, r0:r0 + R, :] = l
        if tied == 2:
            lprev[0] = l
        yield
    LOGITS_STEPS = NW + 3

    def pv_gen(r0, i):
        ls = [pb[w, r0:r0 + RP, :] for w in range(NW)]
        m = functools.reduce(jnp.maximum, ls)
        es = [jnp.exp(l - m) for l in ls]
        yield
        s = functools.reduce(lambda a, b: a + b, es)
        inv = 1.0 / s
        ps = [e * inv for e in es]
        yield
        for c in range(NT):
            acc = None
            for w in range(NW):
                lo = HALO + r0 - DIL * w
                t = ps[w] * vb[c, lo:lo + RP, :]
                acc = t if acc is None else acc + t
            o_all[i * T + r0:i * T + r0 + RP, c * LANES:(c + 1) * LANES] = acc
            yield
    PV_STEPS = NT + 2

    def chain_gens(fns):
        for f in fns:
            yield from f()

    def once(f):
        def g():
            f()
            yield
        return g

    def stream(fns, a=0.0, b=1.0):
        return (chain_gens([once(f) for f in fns]), len(fns), a, b)

    def run_interleaved(mm, streams):
        n = len(mm)
        done = [0] * len(streams)
        for j, fn in enumerate(mm):
            fn()
            for si, (g, steps, a, b) in enumerate(streams):
                frac = min(max(((j + 1) / n - a) / (b - a), 0.0), 1.0)
                target = int(round(frac * steps))
                while done[si] < target:
                    next(g)
                    done[si] += 1
        for g, steps, a, b in streams:
            for _ in g:
                raise AssertionError("stream longer than declared")

    def logits_stream(i, a, b):
        n = T // R
        return (chain_gens([P(logits_gen, j * R, i) for j in range(n)]), n * LOGITS_STEPS, a, b)

    def pv_stream(i, a, b):
        n = T // RP
        return (chain_gens([P(pv_gen, j * RP, i) for j in range(n)]), n * PV_STEPS, a, b)

    def ln1_stream(i, a, b):
        prev[0] = None
        return stream([P(ln1_piece, i, r0, LNR, True) for r0 in range(0, T, LNR)], a, b)

    def wo_piece(c, mi, ki, i):
        cols = slice(c * LANES, (c + 1) * LANES)
        if isinstance(i, int):
            src = pl.ds(i * T + mi * MR, MR)
        else:
            src = pl.ds(pl.multiple_of(i * T + mi * MR, MR), MR)
        lhs = o_all[src, ki * KK:(ki + 1) * KK].astype(bf16)
        r = jnp.dot(lhs, wo[c, ki * KK:(ki + 1) * KK, :], preferred_element_type=f32)
        rs = slice(mi * MR, (mi + 1) * MR)
        if ki == 0:
            hn[rs, cols] = x_all[src, cols].astype(f32) + r
        else:
            hn[rs, cols] += r

    def wo_pieces(i):
        return [P(wo_piece, c, mi, ki, i) for mi in range(T // MR) for c in range(NT) for ki in range(D // KK)]

    def ln2_piece(r0):
        hln[r0:r0 + 32, :] = _layernorm(hn[r0:r0 + 32, :])

    def ffn1_chunk(c):
        cols = slice(c * FC, (c + 1) * FC)
        t = jnp.dot(hln[...].astype(bf16), w1[:, cols], preferred_element_type=f32)
        h1[:, cols] = jnp.maximum(t, 0.0).astype(h1.dtype)

    def ffn2_tile(c, i):
        cols = slice(c * LANES, (c + 1) * LANES)
        t = jnp.dot(h1[...].astype(bf16), w2[:, cols], preferred_element_type=f32)
        out_all[rows(i), cols] = (hc[:, cols] + t).astype(bf16)

    def out_copy(i):
        return pltpu.make_async_copy(out_all.at[rows(i)], out_hbm.at[rows(i)], sem_out)

    def k_halo(src):
        for c in range(NT):
            kb[c, :HALO, :] = src[c, T:, :]

    def v_halo():
        for c in range(NT):
            vb[c, :HALO, :] = vb[c, T:, :]

    LSP = [int(v) for v in "0,0,0,0,4".split(",")]

    def part_logits(lo, hi, a=0.0, b=1.0, tied=0):
        lprev[0] = None
        return (chain_gens([P(logits_gen, j * R, 0, tied) for j in range(lo, hi)]), (hi - lo) * LOGITS_STEPS, a, b)

    def v_first():
        for c in range(NT):
            vb[c, :HALO, :] = jnp.broadcast_to(vb[c, HALO:HALO + 1, :], (HALO, LANES))

    def wo_ts(i):
        return [t for t in range(NT) if 1 + t * (NTILES - 2) // NT == i]

    def step_a(i):
        v_halo()
        streams = [logits_stream(i, 0.0, 1.0)]
        if wo_ts(i):
            streams.append(stream([P(permute_wo, t) for t in wo_ts(i)]))
        run_interleaved(proj_pieces(xn[i % 2], wv, vb, HALO), streams)

    def step_b(i):
        k_halo(k0b if i == 0 else kb)
        x = xn[(i + 1) % 2]
        streams = [pv_stream(i, 0.0, 1.0)]
        if i == 0 and LSP[-1] < T // R:
            streams = [part_logits(LSP[-1], T // R, 0.0, 0.2, 0), pv_stream(i, 0.2, 1.0)]
        if i + 2 < NTILES:
            streams.append(ln1_stream(i + 2, 0.0, 1.0))
        if not 1 and wo_ts(i):
            streams.append(stream([P(permute_wo, t) for t in wo_ts(i)]))
        run_interleaved(proj_pieces(x, wq, qb, 0) + proj_pieces(x, wk, kb, HALO), streams)

    def kpart(xr, w, dst, off, ki):
        return [P(proj_piece, xr, w, dst, off, c, mi, ki) for mi in range(T // MR) for c in range(NT)]

    def block(name, waits, mm, vec):
        for j in waits:
            wait_chain(j)
        if mm:
            region(lambda: run_interleaved(mm, [stream(v) for v in vec]))
        else:
            def plain():
                for v in vec:
                    for f in v:
                        f()
            region(plain)

    pc = lambda g, rb: P(permute_cols, g, rb, (wq, wk, wv)[g])
    assert KK == 512
    for c in range(NT):
        k0b[c, :HALO, :] = jnp.zeros((HALO, LANES), f32)
    x0 = xn[0]
    def chunk_piece(w, dst, off, rb, c2, mi):
        k0 = rb * 256
        lhs = x0[mi * MR:(mi + 1) * MR, k0:k0 + 256].astype(bf16)
        rhs = jnp.concatenate([w[c2, k0:k0 + 256, :], w[c2 + 1, k0:k0 + 256, :]], axis=1)
        r = jnp.dot(lhs, rhs, preferred_element_type=f32)
        rs = slice(off + mi * MR, off + (mi + 1) * MR)
        for j in range(2):
            part = r[:, j * LANES:(j + 1) * LANES]
            if rb == 0:
                dst[c2 + j, rs, :] = part
            else:
                dst[c2 + j, rs, :] += part

    def chunk_mm(n):
        g, rb = divmod(n, 4)
        w, dst, off = ((wq, q0b, 0), (wk, k0b, HALO), (wv, vb, HALO))[g]
        return [P(chunk_piece, w, dst, off, rb, c2, mi) for mi in range(T // MR) for c2 in range(0, NT, 2)]


    pcn = lambda n: pc(n // 4, n % 4)
    block('P0', [0], [], [[P(ln1_piece, 0, r0, 32, False) for r0 in range(0, T, 32)]])
    block('P1', [1], [], [[pcn(0)]])
    for n in range(12):
        if n < 7:
            wait_chain(2 + n)
        elif n == 7:
            wait_chain(9)
            wait_chain(10)
        elif n < 11:
            wait_chain(3 + n)
        def blk(n=n):
            st = []
            if n < 11:
                st.append(stream([pc((n + 1) // 4, (n + 1) % 4)]))
            if n >= 8:
                st.append(part_logits(LSP[n - 8], LSP[n - 7]))
            if n == 11:
                st.append(stream([P(ln1_piece, 1, r0, 32, False) for r0 in range(0, T, 32)]))
            run_interleaved(chunk_mm(n) + ([v_first] if n == 11 else []), st)
        region(blk)
    wait_chain(14)
    assert state["started"] == len(chain)

    for i in range(NTILES):
        cps = []
        if i < NTILES - 1:
            cps = bulk_copies(i) + ([x_copy(i + 3)] if i + 3 < NTILES else [])
            cps += [wo_copy(t) for t in range(NT) if (t * (NTILES - 2) // NT) == i]
        for cp in cps:
            cp.start()
        if i > 0:
            region(P(step_a, i))
        if i < NTILES - 1:
            region(P(step_b, i))
        if i + 3 < NTILES:
            x_copy(i + 3).wait()
        for t in range(NT):
            if i < NTILES - 1 and (t * (NTILES - 2) // NT) == i:
                wo_copy(t).wait()

    last = NTILES - 1

    def last_block():
        wp = wo_pieces(0)
        half = len(wp) // 2
        mm = wp[:half + 2] + [P(ln2_piece, r0) for r0 in range(0, T // 2, 32)] + wp[half + 2:] + [P(ln2_piece, r0) for r0 in range(T // 2, T, 32)]
        run_interleaved(mm, [pv_stream(last, 0.0, 0.75)])
    region(last_block)

    pltpu.make_async_copy(w1_hbm, w1, sem_w.at[12]).wait()
    pltpu.make_async_copy(w2_hbm, w2, sem_w.at[13]).wait()

    def body2(i, carry):
        hc[...] = hn[...]
        for c in range(F // FC):
            ffn1_chunk(c)
        for f in wo_pieces(i + 1):
            f()
        for r0 in range(0, T, 32):
            ln2_piece(r0)
        for c in range(NT):
            ffn2_tile(c, i)
        out_copy(i).start()
        return carry

    lax.fori_loop(0, NTILES - 1, body2, None)
    def epi1():
        hc[...] = hn[...]
        for c in range(F // FC):
            ffn1_chunk(c)
        for c in range(NT - TAILC):
            ffn2_tile(c, last)
    TAILC = 1
    region(epi1)
    split = (NT - TAILC) * LANES
    def part(lo, n):
        cols = pl.ds(lo, n)
        return pltpu.make_async_copy(out_all.at[rows(last), cols], out_hbm.at[rows(last), cols], sem_out)
    part(0, split).start()
    for c in range(NT - TAILC, NT):
        ffn2_tile(c, last)
    part(split, D - split).start()
    pltpu.make_async_copy(out_all, out_hbm, sem_out).wait()


def fused(x, wqkv, wo, w1, w2):
    f32 = jnp.float32
    bf16 = jnp.bfloat16
    any_spec = pl.BlockSpec(memory_space=pl.ANY)
    scratch = [
        pltpu.VMEM((S, D), bf16),
        pltpu.VMEM((3, D, D), bf16),
        pltpu.VMEM((NT, D, LANES), bf16),
        pltpu.VMEM((4, H * PITCH, LANES), jnp.int32),
        pltpu.VMEM((NT, D, LANES), bf16),
        pltpu.VMEM((NT, D, LANES), bf16),
        pltpu.VMEM((NT, D, LANES), bf16),
        pltpu.VMEM((NT, D, LANES), bf16),
        pltpu.VMEM((D, F), bf16),
        pltpu.VMEM((F, D), bf16),
        pltpu.VMEM((T, D), f32),
        pltpu.VMEM((T, D), f32),
        pltpu.VMEM((NT, T, LANES), f32),
        pltpu.VMEM((NT, HALO + T, LANES), f32),
        pltpu.VMEM((NT, T, LANES), f32),
        pltpu.VMEM((NT, HALO + T, LANES), f32),
        pltpu.VMEM((NT, HALO + T, LANES), f32),
        pltpu.VMEM((NW, T, LANES), f32),
        pltpu.VMEM((S, D), f32),
        pltpu.VMEM((T, D), f32),
        pltpu.VMEM((T, D), f32),
        pltpu.VMEM((T, D), f32),
        pltpu.VMEM((T, F), f32),
        pltpu.VMEM((S, D), bf16),
        pltpu.SemaphoreType.DMA((NTILES,)),
        pltpu.SemaphoreType.DMA((22,)),
        pltpu.SemaphoreType.DMA(()),
    ]
    return pl.pallas_call(
        _kernel,
        out_shape=jax.ShapeDtypeStruct((S, D), bf16),
        in_specs=[pl.BlockSpec(memory_space=pltpu.SMEM)] + [any_spec] * 5,
        out_specs=any_spec,
        scratch_shapes=scratch,
        compiler_params=pltpu.CompilerParams(vmem_limit_bytes=110 * 2 ** 20),
        name="fused_block",
    )(np.zeros((1,), np.int32), x, wqkv, wo, w1, w2)


@jax.jit
def pallas_sequential_preLN__sliding_local_dilated__dense_activation_relu__prompt_kernel(
        A_x, A_wqkv, A_wo, B_x, B_w1, B_w2):
    del B_x
    out = fused(A_x.reshape(S, D), A_wqkv, A_wo, B_w1, B_w2)
    return out.reshape(A_x.shape)
```
